```python
import os as _os
_os.environ.setdefault("JAX_PLATFORMS", "cpu")
import jax
import jax.numpy as jnp

def _softmax(x, axis=-1):
    return jax.nn.softmax(x, axis=axis)
def _gelu(x):
    return jax.nn.gelu(x, approximate=True)
def _silu(x):
    return jax.nn.silu(x)
def _sigmoid(x):
    return jax.nn.sigmoid(x)
def _layernorm(x, axis=-1, eps=1e-5):
    m = jnp.mean(x, axis=axis, keepdims=True)
    v = jnp.var(x, axis=axis, keepdims=True)
    return (x - m) / jnp.sqrt(v + eps)
def _scatter_add(tgt, idx, src, axis=0):
    return tgt.at[idx].add(src)
def _segment_sum(src, seg, n):
    return jax.ops.segment_sum(src, seg, n)
class _Rng:
    def __init__(self, key):
        self._k = key
    def _next(self):
        self._k, sub = jax.random.split(self._k)
        return sub
    def normal(self, shape):
        return jax.random.normal(self._next(), shape, dtype=jnp.bfloat16)
    def randint(self, lo, hi, shape):
        return jax.random.randint(self._next(), shape, lo, hi, dtype=jnp.int32)
    def uniform(self, shape, lo=0.0, hi=1.0):
        return jax.random.uniform(self._next(), shape, jnp.bfloat16, lo, hi)
    def permutation(self, n):
        return jax.random.permutation(self._next(), n)


kernel_name = 'gated_mix__ssm_conv_s5__glu_gated_geglu__prompt'

def setup_inputs():
    _rng = _Rng(jax.random.key(int.from_bytes(__import__("os").urandom(4), "little")))
    _w = (lambda a: (lambda t: t.astype(jnp.bfloat16) if jnp.issubdtype(t.dtype, jnp.floating) else t)(jnp.asarray(a)))
    def _A_setup():
        B, S, D = 1, 2048, 1024
        P = D
        Lambda_re = -0.5 * jnp.exp((lambda *s: _rng.normal(s) * 0.4)(P))
        Lambda_im = (lambda *s: _rng.normal(s) * 0.4)(P) * 1.0
        B_re = (lambda *s: _rng.normal(s) * 0.4)(P, D) * (D ** -0.5)
        B_im = (lambda *s: _rng.normal(s) * 0.4)(P, D) * (D ** -0.5)
        C_re = (lambda *s: _rng.normal(s) * 0.4)(D, P) * (P ** -0.5)
        C_im = (lambda *s: _rng.normal(s) * 0.4)(D, P) * (P ** -0.5)
        log_dt = (lambda *s: _rng.normal(s) * 0.4)(P) * 0.3 - 2.0
        Dskip = (lambda *s: _rng.normal(s) * 0.4)(D)
        return {
            "x": _w((lambda *s: _rng.normal(s) * 0.05)(B, S, D)),
            "Lambda_re": _w(Lambda_re),
            "Lambda_im": _w(Lambda_im),
            "B_re": _w(B_re),
            "B_im": _w(B_im),
            "C_re": _w(C_re),
            "C_im": _w(C_im),
            "log_dt": _w(log_dt),
            "Dskip": _w(Dskip),
        }
    _A_in = _A_setup()

    def _B_setup():
        B, S, Dm, Df = 1, 2048, 1024, 3584
        return {
            "x": _w((lambda *s: _rng.normal(s) * 0.05)(B, S, Dm)),
            "w_gate": _w((lambda *s: _rng.normal(s) * 1.6)(Dm, Df) * (Dm ** -0.5)),
            "w_up": _w((lambda *s: _rng.normal(s) * 1.6)(Dm, Df) * (Dm ** -0.5)),
            "w_down": _w((lambda *s: _rng.normal(s) * 1.6)(Df, Dm) * (Df ** -0.5)),
        }
    _B_in = _B_setup()

    return {
        "A_x": _A_in["x"],
        "A_Lambda_re": _A_in["Lambda_re"],
        "A_Lambda_im": _A_in["Lambda_im"],
        "A_B_re": _A_in["B_re"],
        "A_B_im": _A_in["B_im"],
        "A_C_re": _A_in["C_re"],
        "A_C_im": _A_in["C_im"],
        "A_log_dt": _A_in["log_dt"],
        "A_Dskip": _A_in["Dskip"],
        "B_x": _B_in["x"],
        "B_w_gate": _B_in["w_gate"],
        "B_w_up": _B_in["w_up"],
        "B_w_down": _B_in["w_down"],
        "gate_w": _w((lambda *s: _rng.normal(s) * 0.05)(1024) * 16.0),
    }

def reference(A_x, A_Lambda_re, A_Lambda_im, A_B_re, A_B_im, A_C_re, A_C_im, A_log_dt, A_Dskip, B_x, B_w_gate, B_w_up, B_w_down, gate_w):
    def _A_ref(x, Lambda_re, Lambda_im, B_re, B_im, C_re, C_im, log_dt, Dskip):
        Bsz, L, H = x.shape
        Lam = Lambda_re + 1j * Lambda_im
        Bmat = B_re + 1j * B_im
        Cmat = C_re + 1j * C_im
        dt = jnp.exp(log_dt)
        Lam_bar = jnp.exp(dt * Lam)
        B_bar = ((Lam_bar - 1.0) / Lam)[:, None] * Bmat
        Bu = jnp.einsum("bld,pd->blp", x + 0j, B_bar)
        h = jnp.zeros_like(Bu[:, 0, :])
        hs = []
        for t in range(L):
            h = Lam_bar[None, :] * h + Bu[:, t, :]
            hs.append(h)
        hseq = jnp.stack(hs, 1)
        y = 2.0 * jnp.einsum("blp,dp->bld", hseq, Cmat).real + x * Dskip[None, None, :]
        return y

    def _B_ref(x, w_gate, w_up, w_down):
        g = jnp.einsum("bsd,df->bsf", x, w_gate)
        u = jnp.einsum("bsd,df->bsf", x, w_up)
        h = _gelu(g) * u
        return jnp.einsum("bsf,fd->bsd", h, w_down)

    x = A_x
    g = _sigmoid((x * gate_w).sum(-1, keepdims=True))
    a = _A_ref(x, A_Lambda_re, A_Lambda_im, A_B_re, A_B_im, A_C_re, A_C_im, A_log_dt, A_Dskip)
    b = _B_ref(x, B_w_gate, B_w_up, B_w_down)
    return g * a + (1 - g) * b
```

```python
import functools

import jax
import jax.numpy as jnp
from jax import lax
import jax.experimental.pallas as pl
import jax.experimental.pallas.tpu as pltpu

_T = 512
_TF = 512


def _gelu_tanh(g):
    c = 0.7978845608028654
    return 0.5 * g * (1.0 + jnp.tanh(c * (g + 0.044715 * (g * g * g))))


def _ssm_params(lam_re, lam_im, log_dt):
    lam_re = lam_re.astype(jnp.float32)
    lam_im = lam_im.astype(jnp.float32)
    dt = jnp.exp(log_dt.astype(jnp.float32)).astype(jnp.bfloat16).astype(jnp.float32)
    mag = jnp.exp(dt * lam_re)
    ang = dt * lam_im
    a_re = mag * jnp.cos(ang)
    a_im = mag * jnp.sin(ang)
    den = lam_re * lam_re + lam_im * lam_im
    n_re = a_re - 1.0
    c_re = (n_re * lam_re + a_im * lam_im) / den
    c_im = (a_im * lam_re - n_re * lam_im) / den
    return a_re, a_im, c_re, c_im


def _kernel(x_ref, lre8, lim8, ldt8, lre1, lim1, ldt1, dskip_ref, gw_ref,
            bre_hbm, bim_hbm, cre_hbm, cim_hbm, wg_hbm, wu_hbm, wd_hbm,
            o_ref,
            b_s, cre_s, cim_s, cs_s, wg_s, wu_s, wd_s,
            bur_s, bui_s, h_s, hb_s, acc_s, sems,
            *, T, TF, NF, P, D):
    step = pl.program_id(0)

    def b_copy(k):
        src = bre_hbm if k == 0 else bim_hbm
        return pltpu.make_async_copy(src, b_s.at[pl.ds(k * P, P), :], sems.at[k])

    def c_copy(k):
        src, dst = (cre_hbm, cre_s) if k == 0 else (cim_hbm, cim_s)
        return pltpu.make_async_copy(src, dst, sems.at[2 + k])

    def wg_copy(f):
        return pltpu.make_async_copy(wg_hbm.at[:, pl.ds(f * TF, TF)], wg_s.at[f], sems.at[4 + f])

    def wu_copy(f):
        return pltpu.make_async_copy(wu_hbm.at[:, pl.ds(f * TF, TF)], wu_s.at[f], sems.at[4 + NF + f])

    def wd_copy(f):
        return pltpu.make_async_copy(wd_hbm.at[pl.ds(f * TF, TF), :], wd_s.at[f], sems.at[4 + 2 * NF + f])

    @pl.when(step == 0)
    def _():
        b_copy(0).start()
        b_copy(1).start()
        c_copy(0).start()
        c_copy(1).start()
        for f in range(NF):
            wg_copy(f).start()
            wu_copy(f).start()
            wd_copy(f).start()
        h_s[...] = jnp.zeros(h_s.shape, jnp.float32)

    x = x_ref[...]

    @pl.when(step == 0)
    def _():
        b_copy(0).wait()
        b_copy(1).wait()

    bu = lax.dot_general(x, b_s[...], (((1,), (1,)), ((), ())),
                         preferred_element_type=jnp.float32)
    for c in range(P // 128):
        bur_s[pl.ds(c, T, stride=8), :] = bu[:, c * 128:(c + 1) * 128]
        bui_s[pl.ds(c, T, stride=8), :] = bu[:, P + c * 128:P + (c + 1) * 128]

    a_re, a_im, _, _ = _ssm_params(lre8[...], lim8[...], ldt8[...])

    def scan_body(t, carry):
        hr, hi = carry
        r = pl.multiple_of(t * 8, 8)
        br = bur_s[pl.ds(r, 8), :]
        bi = bui_s[pl.ds(r, 8), :]
        nr = a_re * hr - a_im * hi + br
        ni = a_re * hi + a_im * hr + bi
        bur_s[pl.ds(r, 8), :] = nr
        bui_s[pl.ds(r, 8), :] = ni
        return nr, ni

    hr, hi = lax.fori_loop(0, T, scan_body, (h_s[0], h_s[1]), unroll=8)
    h_s[0] = hr
    h_s[1] = hi

    for c in range(P // 128):
        hb_s[:, c * 128:(c + 1) * 128] = bur_s[pl.ds(c, T, stride=8), :].astype(jnp.bfloat16)
        hb_s[:, P + c * 128:P + (c + 1) * 128] = bui_s[pl.ds(c, T, stride=8), :].astype(jnp.bfloat16)

    @pl.when(step == 0)
    def _():
        c_copy(0).wait()
        c_copy(1).wait()
        _, _, c_re, c_im = _ssm_params(lre1[...], lim1[...], ldt1[...])
        cr = cre_s[...].astype(jnp.float32)
        ci = cim_s[...].astype(jnp.float32)
        cs_s[:, 0:P] = (2.0 * (cr * c_re - ci * c_im)).astype(jnp.bfloat16)
        cs_s[:, P:2 * P] = (-2.0 * (cr * c_im + ci * c_re)).astype(jnp.bfloat16)

    y = lax.dot_general(hb_s[...], cs_s[...], (((1,), (1,)), ((), ())),
                        preferred_element_type=jnp.float32)
    xf = x.astype(jnp.float32)
    a = y + xf * dskip_ref[...].astype(jnp.float32)
    gate = jax.nn.sigmoid(jnp.sum(xf * gw_ref[...].astype(jnp.float32), axis=-1, keepdims=True))
    o_ref[...] = gate * a

    def glu_body(f, _):
        @pl.when(step == 0)
        def _():
            wg_copy(f).wait()
            wu_copy(f).wait()
            wd_copy(f).wait()

        g = jnp.dot(x, wg_s[f], preferred_element_type=jnp.float32)
        u = jnp.dot(x, wu_s[f], preferred_element_type=jnp.float32)
        h = (_gelu_tanh(g) * u).astype(jnp.bfloat16)
        d = jnp.dot(h, wd_s[f], preferred_element_type=jnp.float32)

        @pl.when(f == 0)
        def _():
            acc_s[...] = d

        @pl.when(f > 0)
        def _():
            acc_s[...] += d
        return 0

    lax.fori_loop(0, NF, glu_body, 0)
    o_ref[...] += (1.0 - gate) * acc_s[...]


@jax.jit
def pallas_gated_mix__ssm_conv_s5__glu_gated_geglu__prompt_kernel(
    A_x: jax.Array,
    A_Lambda_re: jax.Array,
    A_Lambda_im: jax.Array,
    A_B_re: jax.Array,
    A_B_im: jax.Array,
    A_C_re: jax.Array,
    A_C_im: jax.Array,
    A_log_dt: jax.Array,
    A_Dskip: jax.Array,
    B_x: jax.Array,
    B_w_gate: jax.Array,
    B_w_up: jax.Array,
    B_w_down: jax.Array,
    gate_w: jax.Array,
):
    Bsz, L, D = A_x.shape
    P = A_Lambda_re.shape[0]
    Df = B_w_gate.shape[1]
    T, TF = _T, _TF
    NF = Df // TF
    assert Bsz == 1 and L % T == 0 and Df % TF == 0 and P % 1024 == 0 and P == 1024

    x2 = A_x.reshape(L, D)
    small8 = [v.reshape(8, P // 8) for v in (A_Lambda_re, A_Lambda_im, A_log_dt)]
    small1 = [v.reshape(1, P) for v in (A_Lambda_re, A_Lambda_im, A_log_dt)]
    dskip = A_Dskip.reshape(1, D)
    gw = gate_w.reshape(1, D)

    kernel = functools.partial(_kernel, T=T, TF=TF, NF=NF, P=P, D=D)
    full = lambda shape: pl.BlockSpec(shape, lambda i: (0,) * len(shape))
    anyspec = pl.BlockSpec(memory_space=pl.ANY)

    out = pl.pallas_call(
        kernel,
        grid=(L // T,),
        in_specs=[pl.BlockSpec((T, D), lambda i: (i, 0))]
        + [full((8, P // 8))] * 3 + [full((1, P))] * 3 + [full((1, D))] * 2
        + [anyspec] * 7,
        out_specs=pl.BlockSpec((T, D), lambda i: (i, 0)),
        out_shape=jax.ShapeDtypeStruct((L, D), jnp.float32),
        scratch_shapes=[
            pltpu.VMEM((2 * P, D), jnp.bfloat16),
            pltpu.VMEM((D, P), jnp.bfloat16),
            pltpu.VMEM((D, P), jnp.bfloat16),
            pltpu.VMEM((D, 2 * P), jnp.bfloat16),
            pltpu.VMEM((NF, D, TF), jnp.bfloat16),
            pltpu.VMEM((NF, D, TF), jnp.bfloat16),
            pltpu.VMEM((NF, TF, D), jnp.bfloat16),
            pltpu.VMEM((T * 8, 128), jnp.float32),
            pltpu.VMEM((T * 8, 128), jnp.float32),
            pltpu.VMEM((2, 8, 128), jnp.float32),
            pltpu.VMEM((T, 2 * P), jnp.bfloat16),
            pltpu.VMEM((T, D), jnp.float32),
            pltpu.SemaphoreType.DMA((4 + 3 * NF,)),
        ],
        compiler_params=pltpu.CompilerParams(
            dimension_semantics=("arbitrary",),
            vmem_limit_bytes=100 * 1024 * 1024,
        ),
    )(x2, *small8, *small1, dskip, gw,
      A_B_re, A_B_im, A_C_re, A_C_im, B_w_gate, B_w_up, B_w_down)
    return out.reshape(Bsz, L, D)
```

```python
import functools

import jax
import jax.numpy as jnp
from jax import lax
import jax.experimental.pallas as pl
import jax.experimental.pallas.tpu as pltpu

_T = 512
_TF = 512
_NB = 4
_NO = 4


def _gelu_tanh(g):
    c = 0.7978845608028654
    return 0.5 * g * (1.0 + jnp.tanh(c * (g + 0.044715 * (g * g * g))))


def _kernel(lre_ref, lim_ref, ldt_ref, dskip_ref, gw_ref,
            x_hbm, bre_hbm, bim_hbm, cre_hbm, cim_hbm, wg_hbm, wu_hbm, wd_hbm,
            o_hbm,
            x_s, b_s, cs_s, wg_s, wu_s, wd_s,
            bu_s, h_s, a_s, c_s, hb_s, acc_s, o_s, sems,
            *, T, TF, NF, NB, NO, NS, P, D):
    step = pl.program_id(0)
    PB = 2 * P // NB
    NC = P // 128
    CPB = PB // 128
    NSEG = NF + 1
    SEG = T // NSEG
    TB = T // NB
    DO = D // NO
    always = step >= 0

    s_b, s_c, s_wg, s_wu, s_wd = 0, NB, NB + 2, NB + 2 + NF, NB + 2 + 2 * NF
    s_x = NB + 2 + 3 * NF
    s_o = s_x + NS

    def x_copy(i):
        return pltpu.make_async_copy(x_hbm.at[pl.ds(i * T, T), :], x_s.at[i], sems.at[s_x + i])

    def b_copy(k):
        half = NB // 2
        src = bre_hbm if k < half else bim_hbm
        kk = k % half
        return pltpu.make_async_copy(src.at[pl.ds(kk * PB, PB), :], b_s.at[k], sems.at[s_b + k])

    def b_wait(k):
        return pltpu.make_async_copy(bre_hbm.at[pl.ds(0, PB), :], b_s.at[k], sems.at[s_b + k]).wait()

    def c_copy(k):
        src = cre_hbm if k == 0 else cim_hbm
        return pltpu.make_async_copy(src, cs_s.at[:, pl.ds(k * P, P)], sems.at[s_c + k])

    def wg_copy(f):
        return pltpu.make_async_copy(wg_hbm.at[:, pl.ds(f * TF, TF)], wg_s.at[f], sems.at[s_wg + f])

    def wu_copy(f):
        return pltpu.make_async_copy(wu_hbm.at[:, pl.ds(f * TF, TF)], wu_s.at[f], sems.at[s_wu + f])

    def wd_copy(f):
        return pltpu.make_async_copy(wd_hbm.at[pl.ds(f * TF, TF), :], wd_s.at[f], sems.at[s_wd + f])

    def o_copy(i, n):
        return pltpu.make_async_copy(o_s.at[:, pl.ds(n * DO, DO)],
                                     o_hbm.at[pl.ds(i * T, T), pl.ds(n * DO, DO)], sems.at[s_o + n])

    @pl.when(step == 0)
    def _():
        x_copy(0).start()
        for k in range(NB):
            b_copy(k).start()
        for f in range(NF):
            wg_copy(f).start()
            wu_copy(f).start()
            wd_copy(f).start()
        c_copy(0).start()
        c_copy(1).start()
        for i in range(1, NS):
            x_copy(i).start()
        h_s[...] = jnp.zeros(h_s.shape, jnp.float32)
        lam_re = lre_ref[...].reshape(1, P).astype(jnp.float32)
        lam_im = lim_ref[...].reshape(1, P).astype(jnp.float32)
        log_dt = ldt_ref[...].reshape(1, P).astype(jnp.float32)
        dt = jnp.exp(log_dt).astype(jnp.bfloat16).astype(jnp.float32)
        mag = jnp.exp(dt * lam_re)
        ang = dt * lam_im
        a_re = mag * jnp.cos(ang)
        a_im = mag * jnp.sin(ang)
        den = lam_re * lam_re + lam_im * lam_im
        n_re = a_re - 1.0
        c_s[0] = 2.0 * ((n_re * lam_re + a_im * lam_im) / den)
        c_s[1] = 2.0 * ((a_im * lam_re - n_re * lam_im) / den)
        for c in range(NC):
            a_s[0, c:c + 1, :] = a_re[:, c * 128:(c + 1) * 128]
            a_s[1, c:c + 1, :] = a_im[:, c * 128:(c + 1) * 128]

    x_copy(step).wait()
    x_ref = x_s.at[step]

    def bu_piece(k):
        bu = lax.dot_general(x_ref[...], b_s[k], (((1,), (1,)), ((), ())),
                             preferred_element_type=jnp.float32)
        part = (k * CPB) // NC
        cb = (k * CPB) % NC
        for c in range(CPB):
            bu_s[part, pl.ds(cb + c, T, stride=8), :] = bu[:, c * 128:(c + 1) * 128]
        acc_s[pl.ds(pl.multiple_of(k * TB, TB), TB), :] = jnp.zeros((TB, D), jnp.float32)

    def bu_body(kp, _):
        @pl.when(step == 0)
        def _():
            b_wait(2 * kp)
            b_wait(2 * kp + 1)

        bu_piece(2 * kp)
        bu_piece(2 * kp + 1)
        return 0

    lax.fori_loop(0, NB // 2, bu_body, 0)

    def scan_steps(t0, n, carry, anchor=None):
        hr, hi = carry
        if anchor is not None:
            hr = jnp.where(always, hr, anchor)
        a_re = a_s[0]
        a_im = a_s[1]
        for k in range(n):
            r = pl.multiple_of((t0 + k) * 8, 8)
            br = bu_s[0, pl.ds(r, 8), :]
            bi = bu_s[1, pl.ds(r, 8), :]
            nr = a_re * hr - a_im * hi + br
            ni = a_re * hi + a_im * hr + bi
            bu_s[0, pl.ds(r, 8), :] = nr
            bu_s[1, pl.ds(r, 8), :] = ni
            hr, hi = nr, ni
        return hr, hi

    def hcast(seg, anchors=None):
        t0 = pl.multiple_of(seg * SEG, SEG)
        for c in range(NC):
            hr = bu_s[0, pl.ds(t0 * 8 + c, SEG, stride=8), :]
            hi = bu_s[1, pl.ds(t0 * 8 + c, SEG, stride=8), :]
            cr = c_s[0, :, c * 128:(c + 1) * 128]
            ci = c_s[1, :, c * 128:(c + 1) * 128]
            if anchors is not None:
                cr = jnp.where(always, cr, anchors[c])
            hb_s[pl.ds(t0, SEG), c * 128:(c + 1) * 128] = (cr * hr - ci * hi).astype(jnp.bfloat16)
            hb_s[pl.ds(t0, SEG), P + c * 128:P + (c + 1) * 128] = (-(cr * hi + ci * hr)).astype(jnp.bfloat16)

    carry = scan_steps(0, SEG, (h_s[0], h_s[1]))

    def glu_wait(f):
        wg_copy(f).wait()
        wu_copy(f).wait()
        wd_copy(f).wait()

    def glu_tile(f, carry):
        Q = SEG // 4
        g = jnp.dot(x_ref[...], wg_s[f], preferred_element_type=jnp.float32)
        carry = scan_steps((f + 1) * SEG, Q, carry, g[0:8, 0:128])
        carry = scan_steps((f + 1) * SEG + Q, Q, carry, g[256:264, 0:128])
        u = jnp.dot(x_ref[...], wu_s[f], preferred_element_type=jnp.float32)
        carry = scan_steps((f + 1) * SEG + 2 * Q, Q, carry, u[0:8, 0:128])
        carry = scan_steps((f + 1) * SEG + 3 * Q, Q, carry, u[256:264, 0:128])
        h = (_gelu_tanh(g) * u).astype(jnp.bfloat16)
        hcast(f, [(g if c < 4 else u)[(c % 4) * 128 + 64:(c % 4) * 128 + 65, 0:128] for c in range(NC)])
        d = jnp.dot(h, wd_s[f], preferred_element_type=jnp.float32)
        acc_s[...] += d
        return carry, d

    def glu_pair(fp, carry):
        @pl.when(step == 0)
        def _():
            glu_wait(2 * fp)
            glu_wait(2 * fp + 1)

        carry, _ = glu_tile(2 * fp, carry)
        carry, _ = glu_tile(2 * fp + 1, carry)
        return carry

    carry = lax.fori_loop(0, NF // 2, glu_pair, carry)

    @pl.when(step == 0)
    def _():
        glu_wait(NF - 1)

    @pl.when(step == 0)
    def _():
        c_copy(0).wait()
        c_copy(1).wait()

    @pl.when(step > 0)
    def _():
        for n in range(NO):
            o_copy(step - 1, n).wait()

    (hr, hi), d = glu_tile(NF - 1, carry)
    h_s[0] = hr
    h_s[1] = hi
    hcast(NF, [d[c * 48:c * 48 + 1, 0:128] for c in range(NC)])

    xf = x_ref[...].astype(jnp.float32)
    gw = gw_ref[...].reshape(1, D).astype(jnp.float32)
    dsk = dskip_ref[...].reshape(1, D).astype(jnp.float32)
    gate = jax.nn.sigmoid(jnp.sum(xf * gw, axis=-1, keepdims=True))
    for n in range(NO):
        cols = slice(n * DO, (n + 1) * DO)
        y = lax.dot_general(hb_s[...], cs_s[cols, :], (((1,), (1,)), ((), ())),
                            preferred_element_type=jnp.float32)
        a = y + xf[:, cols] * dsk[:, cols]
        o_s[:, cols] = gate * a + (1.0 - gate) * acc_s[:, cols]
        o_copy(step, n).start()

    @pl.when(step == NS - 1)
    def _():
        for n in range(NO):
            o_copy(step, n).wait()


@jax.jit
def pallas_gated_mix__ssm_conv_s5__glu_gated_geglu__prompt_kernel(
    A_x, A_Lambda_re, A_Lambda_im, A_B_re, A_B_im, A_C_re, A_C_im, A_log_dt, A_Dskip,
    B_x, B_w_gate, B_w_up, B_w_down, gate_w,
):
    Bsz, L, D = A_x.shape
    P = A_Lambda_re.shape[0]
    Df = B_w_gate.shape[1]
    T, TF, NB, NO = _T, _TF, _NB, _NO
    NF = Df // TF
    NS = L // T
    assert Bsz == 1 and L % T == 0 and Df % TF == 0 and P == 1024 and D == 1024

    x2 = A_x.reshape(L, D)
    kernel = functools.partial(_kernel, T=T, TF=TF, NF=NF, NB=NB, NO=NO, NS=NS, P=P, D=D)
    vec = pl.BlockSpec((P,), lambda i: (0,))
    anyspec = pl.BlockSpec(memory_space=pl.ANY)

    out = pl.pallas_call(
        kernel,
        grid=(NS,),
        in_specs=[vec] * 5 + [anyspec] * 8,
        out_specs=anyspec,
        out_shape=jax.ShapeDtypeStruct((L, D), jnp.float32),
        scratch_shapes=[
            pltpu.VMEM((NS, T, D), jnp.bfloat16),
            pltpu.VMEM((NB, 2 * P // NB, D), jnp.bfloat16),
            pltpu.VMEM((D, 2 * P), jnp.bfloat16),
            pltpu.VMEM((NF, D, TF), jnp.bfloat16),
            pltpu.VMEM((NF, D, TF), jnp.bfloat16),
            pltpu.VMEM((NF, TF, D), jnp.bfloat16),
            pltpu.VMEM((2, T * 8, 128), jnp.float32),
            pltpu.VMEM((2, 8, 128), jnp.float32),
            pltpu.VMEM((2, 8, 128), jnp.float32),
            pltpu.VMEM((2, 1, P), jnp.float32),
            pltpu.VMEM((T, 2 * P), jnp.bfloat16),
            pltpu.VMEM((T, D), jnp.float32),
            pltpu.VMEM((T, D), jnp.float32),
            pltpu.SemaphoreType.DMA((NB + 2 + 3 * NF + NS + NO,)),
        ],
        compiler_params=pltpu.CompilerParams(
            dimension_semantics=("arbitrary",),
            vmem_limit_bytes=100 * 1024 * 1024,
        ),
    )(A_Lambda_re, A_Lambda_im, A_log_dt, A_Dskip, gate_w,
      x2, A_B_re, A_B_im, A_C_re, A_C_im, B_w_gate, B_w_up, B_w_down)
    return out.reshape(Bsz, L, D)
```

```python
import functools

import jax
import jax.numpy as jnp
from jax import lax
import jax.experimental.pallas as pl
import jax.experimental.pallas.tpu as pltpu

_T = 512
_TF = 512
_NB = 4
_NO = 4


def _gelu_tanh(g):
    c = 0.7978845608028654
    return 0.5 * g * (1.0 + jnp.tanh(c * (g + 0.044715 * (g * g * g))))


def _kernel(lre_ref, lim_ref, ldt_ref, dskip_ref, gw_ref,
            x_hbm, bre_hbm, bim_hbm, cre_hbm, cim_hbm, wg_hbm, wu_hbm, wd_hbm,
            o_hbm,
            x_s, b_s, cs_s, wg_s, wu_s, wd_s,
            bu_s, h_s, a_s, c_s, hb_s, acc_s, o_s, sems,
            *, T, TF, NF, NB, NO, NS, P, D):
    step = pl.program_id(0)
    PB = 2 * P // NB
    NC = P // 128
    CPB = PB // 128
    NSEG = NF + 1
    SEG = T // NSEG
    TB = T // NB
    DO = D // NO
    always = step >= 0

    s_b, s_c, s_wg, s_wu, s_wd = 0, NB, NB + 2, NB + 2 + NF, NB + 2 + 2 * NF
    s_x = NB + 2 + 3 * NF
    s_o = s_x + NS

    def x_copy(i):
        return pltpu.make_async_copy(x_hbm.at[pl.ds(i * T, T), :], x_s.at[i], sems.at[s_x + i])

    def b_copy(k):
        half = NB // 2
        src = bre_hbm if k < half else bim_hbm
        kk = k % half
        return pltpu.make_async_copy(src.at[pl.ds(kk * PB, PB), :], b_s.at[k], sems.at[s_b + k])

    def b_wait(k):
        return pltpu.make_async_copy(bre_hbm.at[pl.ds(0, PB), :], b_s.at[k], sems.at[s_b + k]).wait()

    def c_copy(k):
        src = cre_hbm if k == 0 else cim_hbm
        return pltpu.make_async_copy(src, cs_s.at[:, pl.ds(k * P, P)], sems.at[s_c + k])

    def wg_copy(f):
        return pltpu.make_async_copy(wg_hbm.at[:, pl.ds(f * TF, TF)], wg_s.at[f], sems.at[s_wg + f])

    def wu_copy(f):
        return pltpu.make_async_copy(wu_hbm.at[:, pl.ds(f * TF, TF)], wu_s.at[f], sems.at[s_wu + f])

    def wd_copy(f):
        return pltpu.make_async_copy(wd_hbm.at[pl.ds(f * TF, TF), :], wd_s.at[f], sems.at[s_wd + f])

    def o_copy(i, n):
        return pltpu.make_async_copy(o_s.at[:, pl.ds(n * DO, DO)],
                                     o_hbm.at[pl.ds(i * T, T), pl.ds(n * DO, DO)], sems.at[s_o + n])

    @pl.when(step == 0)
    def _():
        x_copy(0).start()
        for k in range(NB):
            b_copy(k).start()
        for f in range(NF):
            wg_copy(f).start()
            wu_copy(f).start()
            wd_copy(f).start()
        c_copy(0).start()
        c_copy(1).start()
        for i in range(1, NS):
            x_copy(i).start()
        h_s[...] = jnp.zeros(h_s.shape, jnp.float32)
        lam_re = lre_ref[...].reshape(1, P).astype(jnp.float32)
        lam_im = lim_ref[...].reshape(1, P).astype(jnp.float32)
        log_dt = ldt_ref[...].reshape(1, P).astype(jnp.float32)
        dt = jnp.exp(log_dt).astype(jnp.bfloat16).astype(jnp.float32)
        mag = jnp.exp(dt * lam_re)
        ang = dt * lam_im
        a_re = mag * jnp.cos(ang)
        a_im = mag * jnp.sin(ang)
        den = lam_re * lam_re + lam_im * lam_im
        n_re = a_re - 1.0
        c_s[0] = 2.0 * ((n_re * lam_re + a_im * lam_im) / den)
        c_s[1] = 2.0 * ((a_im * lam_re - n_re * lam_im) / den)
        for c in range(NC):
            a_s[0, c:c + 1, :] = a_re[:, c * 128:(c + 1) * 128]
            a_s[1, c:c + 1, :] = a_im[:, c * 128:(c + 1) * 128]

    x_copy(step).wait()
    x_ref = x_s.at[step]

    def bu_piece(k):
        bu = lax.dot_general(x_ref[...], b_s[k], (((1,), (1,)), ((), ())),
                             preferred_element_type=jnp.float32)
        part = (k * CPB) // NC
        cb = (k * CPB) % NC
        for c in range(CPB):
            bu_s[part, pl.ds(cb + c, T, stride=8), :] = bu[:, c * 128:(c + 1) * 128]
        acc_s[pl.ds(pl.multiple_of(k * TB, TB), TB), :] = jnp.zeros((TB, D), jnp.float32)

    def bu_body(kp, _):
        @pl.when(step == 0)
        def _():
            b_wait(2 * kp)
            b_wait(2 * kp + 1)

        bu_piece(2 * kp)
        bu_piece(2 * kp + 1)
        return 0

    lax.fori_loop(0, NB // 2, bu_body, 0)

    def scan_steps(t0, n, carry, anchor=None):
        hr, hi = carry
        if anchor is not None:
            hr = jnp.where(always, hr, anchor)
        a_re = a_s[0]
        a_im = a_s[1]
        for k in range(n):
            r = pl.multiple_of((t0 + k) * 8, 8)
            br = bu_s[0, pl.ds(r, 8), :]
            bi = bu_s[1, pl.ds(r, 8), :]
            nr = a_re * hr - a_im * hi + br
            ni = a_re * hi + a_im * hr + bi
            bu_s[0, pl.ds(r, 8), :] = nr
            bu_s[1, pl.ds(r, 8), :] = ni
            hr, hi = nr, ni
        return hr, hi

    def hcast(seg, anchors=None):
        t0 = pl.multiple_of(seg * SEG, SEG)
        for c in range(NC):
            hr = bu_s[0, pl.ds(t0 * 8 + c, SEG, stride=8), :]
            hi = bu_s[1, pl.ds(t0 * 8 + c, SEG, stride=8), :]
            cr = c_s[0, :, c * 128:(c + 1) * 128]
            ci = c_s[1, :, c * 128:(c + 1) * 128]
            if anchors is not None:
                cr = jnp.where(always, cr, anchors[c])
            hb_s[pl.ds(t0, SEG), c * 128:(c + 1) * 128] = (cr * hr - ci * hi).astype(jnp.bfloat16)
            hb_s[pl.ds(t0, SEG), P + c * 128:P + (c + 1) * 128] = (-(cr * hi + ci * hr)).astype(jnp.bfloat16)

    carry = scan_steps(0, SEG, (h_s[0], h_s[1]))

    def glu_wait(f):
        wg_copy(f).wait()
        wu_copy(f).wait()
        wd_copy(f).wait()

    def glu_tile(f, carry):
        Q = SEG // 4
        g = jnp.dot(x_ref[...], wg_s[f], preferred_element_type=jnp.float32)
        carry = scan_steps((f + 1) * SEG, Q, carry, g[0:8, 0:128])
        carry = scan_steps((f + 1) * SEG + Q, Q, carry, g[256:264, 0:128])
        u = jnp.dot(x_ref[...], wu_s[f], preferred_element_type=jnp.float32)
        carry = scan_steps((f + 1) * SEG + 2 * Q, Q, carry, u[0:8, 0:128])
        carry = scan_steps((f + 1) * SEG + 3 * Q, Q, carry, u[256:264, 0:128])
        h = (_gelu_tanh(g) * u).astype(jnp.bfloat16)
        hcast(f, [(g if c < 4 else u)[(c % 4) * 128 + 64:(c % 4) * 128 + 65, 0:128] for c in range(NC)])
        d = jnp.dot(h, wd_s[f], preferred_element_type=jnp.float32)
        acc_s[...] += d
        return carry, d

    def glu_pair(fp, carry):
        @pl.when(step == 0)
        def _():
            glu_wait(2 * fp)
            glu_wait(2 * fp + 1)

        carry, _ = glu_tile(2 * fp, carry)
        carry, _ = glu_tile(2 * fp + 1, carry)
        return carry

    carry = lax.fori_loop(0, NF // 2, glu_pair, carry)

    @pl.when(step == 0)
    def _():
        glu_wait(NF - 1)

    @pl.when(step == 0)
    def _():
        c_copy(0).wait()
        c_copy(1).wait()

    @pl.when(step > 0)
    def _():
        for n in range(NO):
            o_copy(step - 1, n).wait()

    (hr, hi), d = glu_tile(NF - 1, carry)
    h_s[0] = hr
    h_s[1] = hi
    hcast(NF, [d[c * 48:c * 48 + 1, 0:128] for c in range(NC)])

    xf = x_ref[...].astype(jnp.float32)
    gw = gw_ref[...].reshape(1, D).astype(jnp.float32)
    dsk = dskip_ref[...].reshape(1, D).astype(jnp.float32)
    gate = jax.nn.sigmoid(jnp.sum(xf * gw, axis=-1, keepdims=True))
    for n in range(NO):
        cols = slice(n * DO, (n + 1) * DO)
        y = lax.dot_general(hb_s[...], cs_s[cols, :], (((1,), (1,)), ((), ())),
                            preferred_element_type=jnp.float32)
        a = y + xf[:, cols] * dsk[:, cols]
        o_s[:, cols] = gate * a + (1.0 - gate) * acc_s[:, cols]
        o_copy(step, n).start()

    @pl.when(step == NS - 1)
    def _():
        for n in range(NO):
            o_copy(step, n).wait()


@jax.jit
def pallas_gated_mix__ssm_conv_s5__glu_gated_geglu__prompt_kernel(
    A_x: jax.Array,
    A_Lambda_re: jax.Array,
    A_Lambda_im: jax.Array,
    A_B_re: jax.Array,
    A_B_im: jax.Array,
    A_C_re: jax.Array,
    A_C_im: jax.Array,
    A_log_dt: jax.Array,
    A_Dskip: jax.Array,
    B_x: jax.Array,
    B_w_gate: jax.Array,
    B_w_up: jax.Array,
    B_w_down: jax.Array,
    gate_w: jax.Array,
):
    Bsz, L, D = A_x.shape
    P = A_Lambda_re.shape[0]
    Df = B_w_gate.shape[1]
    T, TF, NB, NO = _T, _TF, _NB, _NO
    NF = Df // TF
    NS = L // T
    assert Bsz == 1 and L % T == 0 and Df % TF == 0 and P == 1024 and D == 1024

    x2 = A_x.reshape(L, D)
    kernel = functools.partial(_kernel, T=T, TF=TF, NF=NF, NB=NB, NO=NO, NS=NS, P=P, D=D)
    vec = pl.BlockSpec((P,), lambda i: (0,))
    anyspec = pl.BlockSpec(memory_space=pl.ANY)

    out = pl.pallas_call(
        kernel,
        grid=(NS,),
        in_specs=[vec] * 5 + [anyspec] * 8,
        out_specs=anyspec,
        out_shape=jax.ShapeDtypeStruct((L, D), jnp.float32),
        scratch_shapes=[
            pltpu.VMEM((NS, T, D), jnp.bfloat16),
            pltpu.VMEM((NB, 2 * P // NB, D), jnp.bfloat16),
            pltpu.VMEM((D, 2 * P), jnp.bfloat16),
            pltpu.VMEM((NF, D, TF), jnp.bfloat16),
            pltpu.VMEM((NF, D, TF), jnp.bfloat16),
            pltpu.VMEM((NF, TF, D), jnp.bfloat16),
            pltpu.VMEM((2, T * 8, 128), jnp.float32),
            pltpu.VMEM((2, 8, 128), jnp.float32),
            pltpu.VMEM((2, 8, 128), jnp.float32),
            pltpu.VMEM((2, 1, P), jnp.float32),
            pltpu.VMEM((T, 2 * P), jnp.bfloat16),
            pltpu.VMEM((T, D), jnp.float32),
            pltpu.VMEM((T, D), jnp.float32),
            pltpu.SemaphoreType.DMA((NB + 2 + 3 * NF + NS + NO,)),
        ],
        compiler_params=pltpu.CompilerParams(
            dimension_semantics=("arbitrary",),
            vmem_limit_bytes=100 * 1024 * 1024,
        ),
    )(A_Lambda_re, A_Lambda_im, A_log_dt, A_Dskip, gate_w,
      x2, A_B_re, A_B_im, A_C_re, A_C_im, B_w_gate, B_w_up, B_w_down)
    return out.reshape(Bsz, L, D)
```
